```python
import os as _os
_os.environ.setdefault('JAX_PLATFORMS', 'cpu')
import jax
import jax.numpy as jnp

def _softmax(x, axis=-1):
    return jax.nn.softmax(x, axis=axis)

def _gelu(x):
    return jax.nn.gelu(x, approximate=True)

def _silu(x):
    return jax.nn.silu(x)

def _sigmoid(x):
    return jax.nn.sigmoid(x)

def _layernorm(x, axis=-1, eps=1e-05):
    m = jnp.mean(x, axis=axis, keepdims=True)
    v = jnp.var(x, axis=axis, keepdims=True)
    return (x - m) / jnp.sqrt(v + eps)

def _scatter_add(tgt, idx, src, axis=0):
    return tgt.at[idx].add(src)

def _segment_sum(src, seg, n):
    return jax.ops.segment_sum(src, seg, n)

class _Rng:

    def __init__(self, key):
        self._k = key

    def _next(self):
        self._k, sub = jax.random.split(self._k)
        return sub

    def normal(self, shape):
        return jax.random.normal(self._next(), shape, dtype=jnp.bfloat16)

    def randint(self, lo, hi, shape):
        return jax.random.randint(self._next(), shape, lo, hi, dtype=jnp.int32)

    def uniform(self, shape, lo=0.0, hi=1.0):
        return jax.random.uniform(self._next(), shape, jnp.bfloat16, lo, hi)

    def permutation(self, n):
        return jax.random.permutation(self._next(), n)
kernel_name = 'interleave_layers__memory_aug_recurrent_mem_tr__mixer_token_mlp__prompt'

def setup_inputs():
    _rng = _Rng(jax.random.key(int.from_bytes(__import__("os").urandom(4), "little")))
    _w = lambda a: (lambda t: t.astype(jnp.bfloat16) if jnp.issubdtype(t.dtype, jnp.floating) else t)(jnp.asarray(a))

    def _A_setup():
        B, S, Dm = (1, 2048, 640)
        H, Dh = (32, 128)
        M, seg = (8, 32)
        seg = min(seg, S)
        S = S // seg * seg
        return {'x': _w((lambda *s: _rng.normal(s) * 0.05)(B, S, Dm)), 'mem0': _w((lambda *s: _rng.normal(s) * 0.2)(B, M, Dm)), 'Wq': _w((lambda *s: _rng.normal(s) * 0.8)(Dm, H, Dh) * Dm ** (-0.5)), 'Wk': _w((lambda *s: _rng.normal(s) * 0.8)(Dm, H, Dh) * Dm ** (-0.5)), 'Wv': _w((lambda *s: _rng.normal(s) * 0.2)(Dm, H, Dh) * Dm ** (-0.5)), 'Wo': _w((lambda *s: _rng.normal(s) * 0.2)(H, Dh, Dm) * (H * Dh) ** (-0.5)), 'seg_len': seg}
    _A_in = _A_setup()

    def _B_setup():
        B, S, D, F = (1, 2048, 640, 1728)
        return {'x': _w((lambda *s: _rng.normal(s) * 0.05)(B, S, D)), 'w1': _w((lambda *s: _rng.normal(s) * 0.2)(S, F) * S ** (-0.5)), 'b1': _w((lambda *s: _rng.normal(s) * 0.2)(F) * 0.02), 'w2': _w((lambda *s: _rng.normal(s) * 0.2)(F, S) * F ** (-0.5)), 'b2': _w((lambda *s: _rng.normal(s) * 0.2)(S) * 0.02)}
    _B_in = _B_setup()
    return {'A_x': _A_in['x'], 'A_mem0': _A_in['mem0'], 'A_Wq': _A_in['Wq'], 'A_Wk': _A_in['Wk'], 'A_Wv': _A_in['Wv'], 'A_Wo': _A_in['Wo'], 'A_seg_len': _A_in['seg_len'], 'B_x': _B_in['x'], 'B_w1': _B_in['w1'], 'B_b1': _B_in['b1'], 'B_w2': _B_in['w2'], 'B_b2': _B_in['b2']}

def reference(A_x, A_mem0, A_Wq, A_Wk, A_Wv, A_Wo, A_seg_len, B_x, B_w1, B_b1, B_w2, B_b2):

    def _A_ref(x, mem0, Wq, Wk, Wv, Wo, seg_len):
        B, S, Dm = x.shape
        H, Dh = (Wq.shape[1], Wq.shape[2])
        M = mem0.shape[1]
        scale = Dh ** (-0.5)
        n_seg = S // seg_len
        L = M + seg_len
        idx = jnp.arange(L)
        mask = (idx[:, None] < M) | (idx[:, None] >= idx[None, :])
        mem = mem0
        outs = []
        for s in range(n_seg):
            xs = x[:, s * seg_len:(s + 1) * seg_len, :].copy()
            h = jnp.concatenate([mem, xs], axis=1)
            q = jnp.einsum('btd,dhe->bhte', h, Wq)
            k = jnp.einsum('btd,dhe->bhte', h, Wk)
            v = jnp.einsum('btd,dhe->bhte', h, Wv)
            scores = jnp.einsum('bhqe,bhke->bhqk', q, k) * scale
            scores = jnp.where(mask[None, None], scores, -1000000000.0)
            p = _softmax(scores, axis=-1)
            o = jnp.einsum('bhqk,bhke->bhqe', p, v)
            o = jnp.einsum('bhte,hed->btd', o, Wo)
            mem = o[:, :M, :].copy()
            outs.append(o[:, M:, :])
        return jnp.concatenate(outs, axis=1)

    def _B_ref(x, w1, b1, w2, b2):
        B, S, D = x.shape
        h = _layernorm(x, axis=-1)
        u = jnp.einsum('bsd,sf->bdf', h, w1) + b1
        u = _gelu(u)
        y = jnp.einsum('bdf,fs->bds', u, w2) + b2
        return (lambda x, *d: x.transpose(*d))(y, 0, 2, 1)
    x = A_x
    x = x + _A_ref(_layernorm(x, axis=-1), A_mem0, A_Wq, A_Wk, A_Wv, A_Wo, A_seg_len)
    x = x + _B_ref(_layernorm(x, axis=-1), B_w1, B_b1, B_w2, B_b2)
    x = x + _A_ref(_layernorm(x, axis=-1), A_mem0, A_Wq, A_Wk, A_Wv, A_Wo, A_seg_len)
    x = x + _B_ref(_layernorm(x, axis=-1), B_w1, B_b1, B_w2, B_b2)
    return x
```

```python
import functools
import math

import numpy as np
import jax
import jax.numpy as jnp
from jax import lax
import jax.experimental.pallas as pl
import jax.experimental.pallas.tpu as pltpu

F32 = jnp.float32
BF16 = jnp.bfloat16
U32 = jnp.uint32
LOG2E = 1.4426950408889634


def _dot(a, b):
    return lax.dot_general(a, b, (((1,), (0,)), ((), ())), preferred_element_type=F32)


def _dot_nt(a, b):
    return lax.dot_general(a, b, (((1,), (1,)), ((), ())), preferred_element_type=F32)


def _layernorm(x):
    n = x.shape[-1]
    m = jnp.sum(x, axis=-1, keepdims=True) * (1.0 / n)
    d = x - m
    v = jnp.sum(d * d, axis=-1, keepdims=True) * (1.0 / n)
    return d * lax.rsqrt(v + 1e-5)


def _gelu(x):
    c = math.sqrt(2.0 / math.pi)
    return 0.5 * x * (1.0 + jnp.tanh(c * (x + 0.044715 * (x * x * x))))


def default_sched(H, QG, NT):
    ops = []
    ng = H // QG
    att = lambda kind, t: [(kind, h0) for h0 in range(t * QG, (t + 1) * QG)]
    for t in range(ng):
        ops.append(('q', t * QG, QG))
        ops.append(('k', t * QG, QG))
        if t:
            ops += att('pv', t - 1)
        ops.append(('v', t * QG, QG))
        ops += att('s', t)
    he = H - QG
    ops += [('o', 0, 0, he), ('o', 1, 0, he)]
    ops += att('pv', ng - 1)
    ops += [('o', 2, 0, he), ('o', 0, he, H), ('o', 1, he, H), ('o', 2, he, H)]
    ops += [('o', n, 0, H) for n in range(3, NT)]
    return ops


def build(QG=4, unroll1=2, unroll2=4, mb1=432, mb2=512, flags=None, sched=default_sched,
          scopes=False, hdt=F32, rld=16, pm=64, pe=1, dly=0, ahead=2, dsub=128):
    def run(A_x, A_mem0, A_Wq, A_Wk, A_Wv, A_Wo, A_seg_len, B_x, B_w1, B_b1, B_w2, B_b2):
        del B_x
        _, S, D = A_x.shape
        _, H, E = A_Wq.shape
        M = A_mem0.shape[1]
        SEG = int(A_seg_len)
        F = B_w1.shape[1]
        L = M + SEG
        NSEG = S // SEG
        HE = H * E
        NT = D // 128
        scale = float(E) ** -0.5
        HC = 8
        NCH = 3 * H // HC
        PRE = 8
        ops = sched(H, QG, NT)

        class _null:
            def __enter__(self): pass
            def __exit__(self, *a): pass
        scope = (lambda n: jax.named_scope(n)) if scopes else (lambda n: _null())

        def kernel(x_hbm, mem0_ref, wq_hbm, wk_hbm, wv_hbm, wo_hbm, w1_hbm, b1_ref, w2_hbm, b2_ref,
                   out_hbm,
                   xa, xp, xs, hpre, pre, stage, wqkv, wo_in, w1t, w2, w2t, hb, gt, b1c, b2c, xo,
                   sems, wsems, osems, zs):
            zs[0] = 0
            zero = zs[0]
            w_hbm = (wq_hbm, wk_hbm, wv_hbm)
            xp_cp = pltpu.make_async_copy(x_hbm.at[:, pl.ds(SEG - PRE, PRE), :], xp, sems.at[0])
            xa_cp = pltpu.make_async_copy(x_hbm.at[:, pl.ds(0, SEG - PRE), :], xa, sems.at[1])
            wo_cp = pltpu.make_async_copy(wo_hbm, wo_in, sems.at[2])
            w1_cp = pltpu.make_async_copy(w1_hbm, w1t, sems.at[3])
            w2_cp = pltpu.make_async_copy(w2_hbm, w2, sems.at[4])

            def w_cp(i):
                j, c = divmod(i, H // HC)
                return pltpu.make_async_copy(w_hbm[j].at[:, pl.ds(c * HC, HC), :], stage.at[i], wsems.at[i])

            queue = [w_cp(i) for i in range(NCH)] + [xa_cp, wo_cp]
            xp_cp.start()
            for c in queue[:ahead]:
                c.start()

            with scope("init"):
                for c in range(-(-F // 128)):
                    n = min(128, F - c * 128)
                    row = b1_ref[:, pl.ds(c * 128, n)].astype(F32)
                    b1c[pl.ds(c * 128, n), :] = jnp.broadcast_to(row, (128, n)).T
                for c in range(S // 128):
                    row = b2_ref[:, pl.ds(c * 128, 128)].astype(F32)
                    b2c[pl.ds(c * 128, 128), :] = jnp.broadcast_to(row, (128, 128)).T
                xp_cp.wait()
                hpre[...] = _layernorm(xp[...].astype(F32).reshape(NSEG * PRE, D)).astype(hdt)

            def relayout(i, d0, n, z=0):
                w3 = jnp.swapaxes(stage[i, pl.ds(d0, n)], 0, 1)
                for j in range(HC):
                    wqkv[i * HC + z + j, pl.ds(d0 // 2, n // 2), :] = pltpu.bitcast(w3[j], U32)

            with scope("pre"):
                if dly:
                    pl.delay(dly)
                queue[0].wait()
                if ahead < len(queue):
                    queue[ahead].start()
                for j in range(HC):
                    relayout(0, j * D // HC, D // HC)

                def project(i, between):
                    t = 0
                    for m0 in range(0, NSEG * PRE, pm):
                        for j in range(HC):
                            w = pltpu.bitcast(wqkv[i * HC + j], BF16)
                            pre[i * HC + j, pl.ds(m0, pm), :] = _dot(hpre[pl.ds(m0, pm), :], w)
                            if j % pe == pe - 1:
                                between(t)
                                t += 1

                def pre_body(i, c):
                    pltpu.make_async_copy(stage.at[i + 1], stage.at[i + 1], wsems.at[i + 1]).wait()
                    for k in range(NCH - 1):
                        if k + 1 + ahead < len(queue):
                            @pl.when(i == k)
                            def _():
                                queue[k + 1 + ahead].start()

                    def between(t):
                        if t < D // rld:
                            relayout(i + 1, t * rld, rld, i >> 20)

                    project(i, between)
                    return c

                with scope("preloop"):
                    lax.fori_loop(0, NCH - 1, pre_body, 0)
                for c in queue[NCH + ahead:]:
                    c.start()
                xa_cp.wait()
                wo_cp.wait()
                w1_cp.start()
                w2_cp.start()

                def between(t):
                    if t < H:
                        for n in range(NT):
                            wqkv[3 * H + n * 7 + t // NT + zs[0], pl.ds(t % NT * E // 2, E // 2), :] = pltpu.bitcast(
                                wo_in[pl.ds(t * E, E), pl.ds(n * 128, 128)], U32)

                with scope("prelast"):
                    project(NCH - 1, between)

            def a_step(first, s, carry):
                mem, xn = carry
                h = jnp.concatenate([mem, xn], axis=0)
                r = lax.broadcasted_iota(jnp.int32, (L, L), 0)
                c = lax.broadcasted_iota(jnp.int32, (L, L), 1)
                keep = (r < M) | (r >= c)
                pr, ps, o, acc = {}, {}, {}, {}

                sp = jnp.maximum(s - 1, 0)
                sn = jnp.minimum(s + 1, NSEG - 1)
                hb[sp] = _layernorm(_layernorm(xs[sp])).astype(BF16)
                xn_next = _layernorm(xa[sn].astype(F32) if first else xs[sn])

                for op in ops:
                    kind = op[0]
                    if kind in ('q', 'k', 'v'):
                        j = 'qkv'.index(kind)
                        for hh in range(op[1], op[1] + op[2]):
                            y = _dot(h, pltpu.bitcast(wqkv[j * H + hh], BF16))
                            if first:
                                y = jnp.concatenate(
                                    [y, pre[j * H + hh, pl.ds(pl.multiple_of(s * PRE, PRE), PRE), :]], axis=0)
                            pr[kind, hh] = y
                    elif kind == 's':
                        hh = op[1]
                        sc = _dot_nt(pr.pop(('q', hh)), pr.pop(('k', hh)).astype(BF16))
                        sc = jnp.where(keep, sc * (scale * LOG2E), -1e9 * LOG2E)
                        p = jnp.exp2(sc - jnp.max(sc, axis=-1, keepdims=True))
                        l = jnp.sum(p, axis=-1, keepdims=True)
                        rl = pl.reciprocal(l, approx=True)
                        ps[hh] = p, rl * (2.0 - l * rl)
                    elif kind == 'pv':
                        hh = op[1]
                        p, rl = ps.pop(hh)
                        o[hh] = _dot(p, pr.pop(('v', hh)).astype(BF16)) * rl
                    elif kind == 'o':
                        _, n, h0, h1 = op
                        lhs = jnp.concatenate([o[hh] for hh in range(h0, h1)], axis=1)
                        w = jnp.concatenate(
                            [wqkv[3 * H + n * 7 + hh // NT, pl.ds(hh % NT * E // 2, E // 2), :] for hh in range(h0, h1)], axis=0)
                        part = _dot(lhs, pltpu.bitcast(w, BF16))
                        acc[n] = part + acc[n] if n in acc else part
                out = jnp.concatenate([acc[n] for n in range(NT)], axis=1)
                if first:
                    x = jnp.concatenate([xa[s].astype(F32), xp[s].astype(F32)], axis=0)
                else:
                    x = xs[s]
                xs[s] = x + out[M:]
                return out[:M], xn_next

            def layer(li, c):
                mem0 = mem0_ref[...].astype(F32)

                @pl.when(li == 0)
                def _():
                    with scope("A1"):
                        xs[0] = jnp.zeros((SEG, D), F32)
                        lax.fori_loop(0, NSEG, functools.partial(a_step, True),
                                      (mem0, _layernorm(xa[0].astype(F32))), unroll=unroll1)
                    w1_cp.wait()
                    w2_cp.wait()

                @pl.when(li > 0)
                def _():
                    with scope("A2"):
                        lax.fori_loop(0, NSEG, functools.partial(a_step, False),
                                      (mem0, _layernorm(xs[0])), unroll=unroll2)

                hb[NSEG - 1] = _layernorm(_layernorm(xs[NSEG - 1])).astype(BF16)
                nup = F // mb1
                tw = S // nup

                def up(i, c):
                    r = pl.ds(pl.multiple_of(i * mb1, 16), mb1)
                    u = _dot(w1t[r, :], hb[...].reshape(S, D)) + jnp.tile(b1c[r, :], (1, NT))
                    gt[r, :] = _gelu(u).astype(BF16)
                    t = pl.ds(pl.multiple_of(i * tw, tw), tw)
                    w2t[t, :] = w2[:, t].T
                    return c

                with scope("up"):
                    lax.fori_loop(0, nup, up, 0)

                def o_cp(i):
                    r = pl.ds(pl.multiple_of(i * mb2, mb2), mb2)
                    return pltpu.make_async_copy(xo.at[r], out_hbm.at[r], osems.at[i])

                def down(i, c):
                    r = pl.ds(pl.multiple_of(i * mb2, mb2), mb2)
                    g = pl.ds(i * (mb2 // SEG), mb2 // SEG)
                    y = _dot(w2t[r, :], gt[...]) + jnp.tile(b2c[r, :], (1, NT))
                    x = xs[g].reshape(mb2, D) + y
                    xs[g] = x.reshape(mb2 // SEG, SEG, D)
                    xo[r, :] = x.astype(BF16)

                    @pl.when(li == 1)
                    def _():
                        o_cp(i).start()
                    return c

                with scope("down"):
                    lax.fori_loop(0, S // mb2, down, 0)

                @pl.when(li == 1)
                def _():
                    for i in range(S // mb2):
                        o_cp(i).wait()
                return c

            lax.fori_loop(0, 2, layer, 0)

        hbm = pl.BlockSpec(memory_space=pltpu.MemorySpace.HBM)
        vspec = pl.BlockSpec(memory_space=pltpu.VMEM)
        out = pl.pallas_call(
            kernel,
            out_shape=jax.ShapeDtypeStruct((S, D), BF16),
            in_specs=[hbm, vspec, hbm, hbm, hbm, hbm, hbm, vspec, hbm, vspec],
            out_specs=hbm,
            scratch_shapes=[
                pltpu.VMEM((NSEG, SEG - PRE, D), BF16),
                pltpu.VMEM((NSEG, PRE, D), BF16),
                pltpu.VMEM((NSEG, SEG, D), F32),
                pltpu.VMEM((NSEG * PRE, D), hdt),
                pltpu.VMEM((3 * H, NSEG * PRE, E), F32),
                pltpu.VMEM((NCH, D, HC, E), BF16),
                pltpu.VMEM((3 * H + 7 * NT, D // 2, E), U32),
                pltpu.VMEM((HE, D), BF16),
                pltpu.VMEM((F, S), BF16),
                pltpu.VMEM((F, S), BF16),
                pltpu.VMEM((S, F), BF16),
                pltpu.VMEM((NSEG, SEG, D), BF16),
                pltpu.VMEM((F, D), BF16),
                pltpu.VMEM((F, 128), F32),
                pltpu.VMEM((S, 128), F32),
                pltpu.VMEM((S, D), BF16),
                pltpu.SemaphoreType.DMA((5,)),
                pltpu.SemaphoreType.DMA((NCH,)),
                pltpu.SemaphoreType.DMA((S // mb2,)),
                pltpu.SMEM((1,), jnp.int32),
            ],
            compiler_params=pltpu.CompilerParams(vmem_limit_bytes=120 * 1024 * 1024, flags=flags),
            name="rmt",
        )(
            A_x.reshape(NSEG, SEG, D), A_mem0.reshape(M, D),
            A_Wq, A_Wk, A_Wv, A_Wo.reshape(HE, D),
            B_w1.T, B_b1.reshape(1, F), B_w2, B_b2.reshape(1, S),
        )
        return out.reshape(A_x.shape)

    return run


_run = build(unroll1=2, unroll2=2, ahead=3)


def pallas_interleave_layers__memory_aug_recurrent_mem_tr__mixer_token_mlp__prompt_kernel(
        A_x, A_mem0, A_Wq, A_Wk, A_Wv, A_Wo, A_seg_len, B_x, B_w1, B_b1, B_w2, B_b2):
    return _run(A_x, A_mem0, A_Wq, A_Wk, A_Wv, A_Wo, A_seg_len, B_x, B_w1, B_b1, B_w2, B_b2)
```

```python
import functools
import math

import jax
import jax.numpy as jnp
from jax import lax
import jax.experimental.pallas as pl
import jax.experimental.pallas.tpu as pltpu

F32 = jnp.float32
BF16 = jnp.bfloat16
U32 = jnp.uint32
LOG2E = 1.4426950408889634
T, U = 0, 1
SLICES = 8


def _dot(a, b):
    return lax.dot_general(a, b, (((1,), (0,)), ((), ())), preferred_element_type=F32)


def _dot_nt(a, b):
    return lax.dot_general(a, b, (((1,), (1,)), ((), ())), preferred_element_type=F32)


def _layernorm(x):
    n = x.shape[-1]
    d = x - jnp.sum(x, axis=-1, keepdims=True) * (1.0 / n)
    v = jnp.sum(d * d, axis=-1, keepdims=True) * (1.0 / n)
    return d * lax.rsqrt(v + 1e-5)


def _gelu(x):
    c = math.sqrt(2.0 / math.pi)
    return 0.5 * x * (1.0 + jnp.tanh(c * (x + 0.044715 * (x * x * x))))


def _half_word(w, i):
    return lax.bitcast_convert_type(w & jnp.uint32(0xFFFF0000) if i else w << 16, F32)


def _memo(f):
    seen = {}

    def g(*k):
        if k not in seen:
            seen[k] = f(*k)
        return seen[k]

    return g


def _scheme(X, Y, pairs):
    P = {}
    for i, (a, d) in enumerate(X):
        ys = [Y[l] for k, l in pairs if k == i]
        P['m3', i] = ({(T, a): 1}, {(a, d): 1, **{(b, d): -1 for b, _ in ys}}, {(T, d): 1, (U, d): 1})
        P['m6', i] = ({(U, a): 1, (T, a): -1}, {(a, d): 1, **{(a, c): 1 for _, c in ys}}, {(U, d): 1})
    for l, (b, c) in enumerate(Y):
        xs = [X[i] for i, k in pairs if k == l]
        P['m4', l] = ({(U, b): 1}, {(b, c): 1, **{(a, c): -1 for a, _ in xs}}, {(T, c): 1, (U, c): 1})
        P['m7', l] = ({(T, b): 1, (U, b): -1}, {(b, c): 1, **{(b, d): 1 for _, d in xs}}, {(T, c): 1})
    for i, l in pairs:
        (a, d), (b, c) = X[i], Y[l]
        P['m1', i, l] = ({(T, a): 1, (U, b): 1}, {(a, c): 1, (b, d): 1}, {(T, c): 1, (U, d): 1})
        P['m2', i, l] = ({(U, a): 1, (U, b): 1}, {(a, c): 1}, {(U, c): 1, (U, d): -1})
        P['m5', i, l] = ({(T, a): 1, (T, b): 1}, {(b, d): 1}, {(T, c): -1, (T, d): 1})
    return P


HEAD_GROUPS = ((0, 6), (12, 5), (22, 5))
PAIRS = {6: [(i, l) for i in range(6) for l in range(6) if l not in (i, (i + 1) % 6)],
         5: [(i, l) for i in range(5) for l in range(5) if l != i]}
PROJ = [_scheme([(i, h + i) for i in range(n)], [(i, h + n + i) for i in range(n)], PAIRS[n])
        for h, n in HEAD_GROUPS]
OUT = [_scheme([(h + i, i) for i in range(n)], [(h + n + i, i) for i in range(n)], PAIRS[n])
       for h, n in HEAD_GROUPS]
ATTN_TILE = {k: i for i, k in enumerate((g, k) for g, s in enumerate(PROJ) for k in s)}


def _attn_block(v, h):
    r = 5 if h >= 12 else (h + 1) % 6 if h < 6 else (h - 1) % 6
    return {v: 1} if r == 5 else {r: 1} if v == 5 else {v: 1, r: -1}


_DIAG = [(i, i) for i in range(14)]
MIX = _scheme(_DIAG[:7], _DIAG[7:], [(i, l) for i in range(7) for l in range(7)])
MIX_TILE = {k: i for i, k in enumerate(k for k in MIX if k[0] not in ('m2', 'm5') or k[1] == k[2])}
TOKEN_TILE = (0, 1, 2, 3, 4, 5, 7, 6)
MIRROR = {'m1': 'm1', 'm2': 'm5', 'm5': 'm2', 'm3': 'm6', 'm6': 'm3', 'm4': 'm7', 'm7': 'm4'}


def _mix_block(v, f):
    if f < 7:
        return {7: 1} if v == f else {f: 1, 7: -1} if v == f + 7 else {v - 7: 1}
    rest = [k for k in range(7) if k != f - 7]
    if v == f - 7:
        return {7: 1, **{k: -1 for k in rest}}
    return {f - 7: 1, 7: -1, **{k: 1 for k in rest}} if v == f else {v: 1}


def _signed_add(acc, key, sign, val):
    if key not in acc:
        acc[key] = (sign, val)
        return
    s0, v0 = acc[key]
    acc[key] = (s0, v0 + val) if s0 == sign else (1, v0 - val if s0 > 0 else val - v0)


def _take(acc, key):
    s, v = acc[key]
    acc[key] = None
    assert s > 0
    return v


def _combine(terms, get):
    acc = {}
    for k, c in terms.items():
        _signed_add(acc, 0, c, get(k))
    return _take(acc, 0)


def _half_order(ph, n, mode):
    diag, single = (('m3', 'm7'), 'm5') if ph == T else (('m4', 'm6'), 'm2')
    pick = {'column': lambda p: p[ph], 'finish': min, 'open': max}[mode]
    left = [(d, s) for s in range(n) for d in diag]
    keys, done = [], 0
    for s in range(n):
        while mode == 'column' and left and left[0][1] <= s:
            keys.append(left.pop(0))
        for p in sorted((p for p in PAIRS[n] if pick(p) == s), key=lambda p: p[0] != s):
            keys += [(single, *p), ('m1', *p)]
            done += 1
            if mode != 'column' and done % 2 == 0 and left and (mode == 'finish' or left[0][1] <= s):
                keys.append(left.pop(0))
        while left and left[0][1] <= s:
            keys.append(left.pop(0))
    return keys


def _mix_order():
    keys = []
    for s in range(7):
        keys += [(m, s, l) for l in [*range(s + 1, 7), s] for m in ('m1', 'm2', 'm5')] + [('m3', s), ('m6', s)]
        keys += [(m, i, s) for i in range(s + 1, 7) for m in ('m1', 'm2', 'm5')] + [('m4', s), ('m7', s)]
    return keys


def _rounds(jobs):
    queues = [[(i, f) for i, (long, f) in enumerate(jobs) if long == k] for k in (False, True)]
    out = []
    while queues[0] or queues[1]:
        at = [q[min(3, len(q) - 1)][0] if q else math.inf for q in queues]
        q = queues[at[1] < at[0]]
        out += [f for _, f in q[:4]]
        del q[:4]
    return out


def _spread(fill, jobs, lo, hi):
    for i, f in enumerate(jobs):
        at = lo + i * (hi - lo) // len(jobs)
        while at in fill:
            at += 1
        fill[at] = f


HEADS = ((0, 1, 2, 3), (4, 5, 6, 7), (8, 9, 10, 11), (12, 13, 14, 15), (16, 17, 18, 19),
         (20, 21, 22, 27), (23, 28, 24, 29), (25, 30, 26, 31))
SCORES_AT = ((146, 152, 185, 290, 326, 446, 452, 462), (154, 152, 177, 305, 326, 462, 452, 459),
             (157, 152, 192, 305, 326, 444, 452, 462), (164, 152, 185, 305, 326, 446, 466, 462))
VALUES_AT = ((200, 225, 269, 395, 420, 496, 515, 509), (202, 225, 269, 395, 415, 496, 510, 520),
             (202, 225, 269, 395, 410, 487, 510, 520), (200, 225, 269, 385, 410, 496, 510, 517))
LAST_HEADS_LAG = ((65, 68), (76, 68), (65, 88), (65, 84))
SETTLE = ((31, 20), (30, 29), (30, 20), (30, 30))
SIDE_JOBS = (((230, 470), (800, 1135), (130, 542)), ((88, 470), (800, 1100), (22, 501)))
FIRST_VALUES_AT = (112, 136, 160, 208, 232, 0, 0, 0)
COPIES_FIRST, COPIES_AHEAD = 2, 6


@functools.partial(jax.jit, static_argnames=("A_seg_len",))
def pallas_interleave_layers__memory_aug_recurrent_mem_tr__mixer_token_mlp__prompt_kernel(
        A_x, A_mem0, A_Wq, A_Wk, A_Wv, A_Wo, A_seg_len, B_x, B_w1, B_b1, B_w2, B_b2):
    del B_x
    _, S, D = A_x.shape
    _, H, E = A_Wq.shape
    M = A_mem0.shape[1]
    SEG = int(A_seg_len)
    F = B_w1.shape[1]
    L, HALF, NSEG, GB = M + SEG, SEG // 2, S // SEG, 128 // SEG
    NT, NS, NF = D // 128, S // 128, -(-F // 128)
    NW, NB = len(ATTN_TILE), len(MIX_TILE)
    assert (D, H, E, M, SEG, S, NF) == (640, 32, 128, 8, 32, 2048, 14) and F % 16 == 0
    early = [(g, k) for k in range(6) for g in range(2)]
    late_y = (13, 14, 15)

    def proj_passes(ph, j, g):
        mode = 'column'
        if isinstance(j, int):
            mode = 'open' if (j, g) == (0, 0) else 'finish' if j and g == 2 else mode
        return [([(PROJ[g][k][0], NW * j + ATTN_TILE[g, k])], PROJ[g][k][2], k[0] == 'm1')
                for k in _half_order(ph, HEAD_GROUPS[g][1], mode)]

    def out_passes(ph):
        keys = [k for k in _half_order(ph, 6, 'finish') if 5 in k[1:]] + _half_order(ph, 5, 'finish')
        groups = {k: [g for g in range(3) if k in OUT[g]] for k in keys}
        return [([(OUT[g][k][0], 3 * NW + ATTN_TILE[g, k]) for g in gs], OUT[gs[0]][k][2], k[0] == 'm1')
                for k, gs in groups.items()]

    def kernel(x_hbm, mem0_hbm, wq_hbm, wk_hbm, wv_hbm, wo_hbm, w1_hbm, b1_hbm, w2_hbm, b2_hbm, out_hbm,
               mem0, b1, b2, xs, wqkv_in, wo_in, w12, wa, wb, bias, xn, qkv_even, qkv_odd, o_mem,
               o_even0, o_even1, o_odd, hb, h_next, g_buf, y_last, sems, wsems, osems):
        o_even = (o_even0, o_even1)

        def staged(n):
            return wqkv_in.at[n, :, pl.ds(0, 16 * H)]

        def w_cp(j, i):
            n = j * SLICES + i
            if j < 3:
                return pltpu.make_async_copy((wq_hbm, wk_hbm, wv_hbm)[j].at[:, i], staged(n), wsems.at[n])
            return pltpu.make_async_copy(wo_hbm.at[:, i], wo_in.at[i], wsems.at[n])

        def x_cps(i, lo, hi):
            return [pltpu.make_async_copy(x_hbm.at[pl.ds(lo, hi - lo), :, pl.ds(k * 128, 128)],
                                          xs.at[k, pl.ds(lo, hi - lo)], sems.at[NT * i + k]) for k in range(NT)]

        def out_cp(i, part):
            cols = pl.ds(pl.multiple_of(i * 128, 128), 128)
            cut = late_y[0] * GB
            rows = (pl.ds(0, cut), pl.ds(cut, NSEG - cut))[part]
            return pltpu.make_async_copy(xs.at[i, rows], out_hbm.at[rows, :, cols], osems.at[2 * i + part])

        x_head, x_soon, x_rest = x_cps(0, 0, 4), x_cps(1, 4, 8), x_cps(2, 8, NSEG)
        w1_cp, w2_cp, *small = [
            pltpu.make_async_copy(src, dst, sems.at[3 * NT + i]) for i, (src, dst) in enumerate((
                (w1_hbm, w12.at[0, pl.ds(0, F)]), (w2_hbm, w12.at[1, pl.ds(0, F)]),
                (mem0_hbm, mem0), (b1_hbm, b1), (b2_hbm, b2)))]

        def start_all(cps):
            for cp in cps:
                cp.start()

        def wait_all(cps):
            for cp in cps:
                cp.wait()

        def start_ahead(j, i):
            for k in range(4):
                @pl.when((j * SLICES + i + COPIES_AHEAD) // SLICES == k)
                def _():
                    w_cp(k, (i + COPIES_AHEAD) % SLICES).start()

        def weight_sums(m, i, schemes, block):
            def store(g, k, y):
                wa[NW * m + ATTN_TILE[g, k], pl.ds(pl.multiple_of(i * 16, 16), 16), :] = y.astype(BF16)

            for g, (scheme, (_, n)) in enumerate(zip(schemes, HEAD_GROUPS)):
                acc = {}
                for a, b in PAIRS[n]:
                    for name in ('m2', 'm5', 'm1'):
                        store(g, (name, a, b), _combine(scheme[name, a, b][1], lambda k: block(*k)))
                    for k in (('m3', a), ('m6', a), ('m4', b), ('m7', b)):
                        w = scheme[k][1]
                        new = [x for x in w if x in scheme['m1', a, b][1]]
                        for x in new if k in acc else [next(iter(w))] + new:
                            _signed_add(acc, k, w[x], block(*x))
                        if (a, b) == [p for p in PAIRS[n] if p[k[0] in ('m4', 'm7')] == k[1]][-1]:
                            store(g, k, _take(acc, k))

        def prepare_proj(j):
            words = wqkv_in.bitcast(U32)

            def body(i, c):
                n = j * SLICES + i
                pltpu.make_async_copy(staged(n), staged(n), wsems.at[n]).wait()
                pl.when(n == 0)(lambda: start_all(
                    [w_cp(0, k) for k in range(COPIES_FIRST, COPIES_AHEAD)] + x_head))
                start_ahead(j, i)
                word = _memo(lambda k, hp: jnp.concatenate(
                    [words[n, k, pl.ds(r * 4 * H + hp, 8, stride=H // 2), :] for r in range(2)]))
                real = _memo(lambda k, h: _half_word(word(k, h // 2), h % 2))
                weight_sums(j, i, PROJ, _memo(lambda v, h: _combine(_attn_block(v, h), lambda k: real(k, h))))
                return c

            lax.fori_loop(0, SLICES, body, 0)

        def prepare_out():
            def body(i, c):
                w_cp(3, i).wait()
                start_ahead(3, i)
                pl.when(i == 2)(lambda: start_all(x_soon))
                real = _memo(lambda h, n: wo_in[i, h, :, pl.ds(n * 128, 128)].astype(F32))
                weight_sums(3, i, OUT, _memo(lambda h, v: _combine(_attn_block(v, h), lambda n: real(h, n))))
                return c

            lax.fori_loop(0, SLICES, body, 0)
            start_all(x_rest + [w1_cp])

        def prepare_mix(u):
            half, i = jnp.maximum(u, 0) >> 3, jnp.maximum(u, 0) & 7
            sign = lax.convert_element_type((half & 2) - 1, F32)
            src = w12.at[jnp.where(u < 0, 2, half >> 1), pl.ds(pl.multiple_of(i * 16, 16), (NF - 1) * 128 + 16),
                         pl.ds(pl.multiple_of((half & 1) * (S // 2), S // 2), S // 2)]
            dst = wb.at[pl.ds(half * NB, NB), pl.ds(pl.multiple_of(i * 16, 16), 16)]
            word = _memo(lambda k, f: src[pl.ds(f * 128, 16), pl.ds(TOKEN_TILE[k] * 128, 128)])
            block = _memo(lambda v, f: _combine(_mix_block(v, f), lambda k: word(k, f).astype(F32)))

            def job(keys):
                done = []
                for k in keys:
                    (head, _), *tail = MIX[k][1].items()
                    y = block(*head)
                    if tail:
                        z = _combine({b: 1 for b, _ in tail}, lambda b: block(*b))
                        y = y + z if k[0] == 'm1' else y + sign * z if tail[0][1] < 0 else y - sign * z
                    dst[MIX_TILE[k]] = y.astype(BF16)
                    done.append(bits(y))
                return functools.reduce(jnp.bitwise_or, done)

            off = [k for k in MIX_TILE if len(k) == 3 and k[1] != k[2]]
            parts = [p for d in range(7) for p in (
                [(x, d, d) for x in ('m2', 'm5', 'm1')], *[[(x, d)] for x in ('m3', 'm6', 'm4', 'm7')])]
            return [functools.partial(job, p) for p in parts + [off[c:c + 3] for c in range(0, len(off), 3)]]

        def bits(y):
            parts = [y[r:r + 8, c:c + 128] for r in range(0, y.shape[0], 8) for c in sorted({0, y.shape[1] - 128})]
            return functools.reduce(jnp.bitwise_or, [lax.bitcast_convert_type(p, U32) for p in parts])

        def after(y, done, zero):
            return lax.bitcast_convert_type(lax.bitcast_convert_type(y, U32) | (done & zero), F32)

        def tiles_and_sum(y):
            tiles = [y[:, k * 128:(k + 1) * 128] for k in range(NT)]
            return tiles + [functools.reduce(jnp.add, tiles)]

        def real_tiles(get):
            total = get(NT)
            return jnp.concatenate([get(n) + total for n in range(NT)], axis=1)

        def x_tile(k, s, r=0, n=SEG):
            return pltpu.bitcast(xs.bitcast(U32)[k, s, pl.ds(r // 2, n // 2), :], BF16).astype(F32)

        def load_x(s, r, n):
            return jnp.concatenate([x_tile(k, s, r, n) for k in range(NT)], axis=1)

        def attn_in(s, buf, p, r=0, n=SEG):
            y = tiles_and_sum(_layernorm(load_x(s + p, r, n)))
            for k, tile in enumerate(y):
                xn[buf, p, k, pl.ds(r, n), :] = tile
            return bits(y[-1])

        def mixer_in(s, r=0, n=SEG):
            y = _layernorm(_layernorm(load_x(s, r, n)))
            for k in range(NT):
                hb[k, s, pl.ds(r, n), :] = y[:, k * 128:(k + 1) * 128]
            return bits(y)

        def product_jobs(passes, ph, halves, mem_in, tok_in, mem_acc, tok_acc):
            jobs = []
            for terms, out, shared in passes:
                hs = () if tok_in is None else halves if shared else (0, 1)
                if mem_in is None and not hs:
                    continue

                def job(rows_of, tile, count, out, hs, parts):
                    rows = [mem_in({k: c for (p, k), c in rows_of.items() if p == ph})] if mem_in else []
                    rows += [tok_in(rows_of, h) for h in hs]
                    res = _dot(jnp.concatenate(rows), pltpu.bitcast(wa.bitcast(U32)[tile], BF16))
                    parts.append(res + parts[-1] if parts else res)
                    if len(parts) < count:
                        return
                    r0 = M if mem_in else 0
                    for (p, n), c in out.items():
                        if mem_in and p == ph:
                            _signed_add(mem_acc, n, c, parts[-1][:M])
                    for i, h in enumerate(hs):
                        for (p, n), c in out.items():
                            _signed_add(tok_acc, (p, n, h), c, parts[-1][r0 + i * HALF:r0 + (i + 1) * HALF])

                parts = []
                jobs += [(len(hs) > 1, functools.partial(job, *t, len(terms), out, hs, parts)) for t in terms]
            return jobs

        def memory_rows(mem):
            tiles = tiles_and_sum(mem)
            rows = _memo(lambda *l: _combine(dict(l), tiles.__getitem__))
            return lambda l: rows(*sorted(l.items()))

        def token_rows(buf):
            rows = _memo(lambda h, *l: _combine(dict(l), lambda k: xn[buf, k[0], k[1], pl.ds(h * HALF, HALF), :]))
            return lambda l, h: rows(h, *sorted(l.items()))

        def both(acc, p, n):
            return jnp.concatenate([_take(acc, (p, n, i)) for i in range(2)])

        def probs(q, k):
            sc = _dot_nt(q, k.astype(BF16)) * (E ** -0.5 * LOG2E)
            r = lax.broadcasted_iota(jnp.int32, (L, L), 0)
            c = lax.broadcasted_iota(jnp.int32, (L, L), 1)
            sc = jnp.where(((r < M) | (r >= c))[L - q.shape[0]:], sc, -1e9 * LOG2E)
            p = jnp.exp2(sc - jnp.max(sc, axis=-1, keepdims=True))
            total = jnp.sum(p, axis=-1, keepdims=True)
            inv = pltpu.reciprocal(total, approx=True)
            return p, inv * (2.0 - total * inv)

        def step(ph, mem, buf, tok_p, p_acc, o_halves, o_acc, fill, zero, carried, last=False):
            tune = 2 * buf + ph
            o_tok, o_dst = (o_even[1 - buf], o_odd), (o_even[buf], o_odd)[ph]
            m_acc, ps, seen, due = [{}, {}, {}, {}], {}, set(), []
            now = [0]
            mem_in = memory_rows(mem)

            def ordered(y):
                for e in [e for e in due if e[0] <= now[0]]:
                    y = after(y, e[1], zero)
                due[:] = [e for e in due if e[0] > now[0]]
                return y

            def mem_o(l):
                assert seen.issuperset(l)
                return ordered(_combine(l, lambda h: o_mem[h]))

            def tok_o(l, i):
                assert seen.issuperset(h for p, h in l if p == U == ph)
                return _combine(l, lambda k: o_tok[k[0]][k[1], pl.ds(i * HALF, HALF), :])

            def qkv(j, h):
                rows = [_take(m_acc[j], h)] if j or not last else []
                if ph == T:
                    return jnp.concatenate(rows + [both(p_acc[j], T, h)])
                return jnp.concatenate(rows + [carried.pop((j, h)) if carried else qkv_odd[j * H + h]])

            def scores(h):
                ps[h] = probs(qkv(0, h), qkv(1, h))

            def values(h):
                p, inv = ps.pop(h)
                y = _dot(p, qkv(2, h).astype(BF16)) * inv
                o_dst[h] = y[-SEG:]
                seen.add(h)
                if last:
                    return
                o_mem[h] = y[:M]
                if len(seen) % 4 == 0 and len(seen) <= SETTLE[tune][1]:
                    for ref in (o_dst, o_mem):
                        due.append((now[0] + SETTLE[tune][0], bits(ref[h + zero.astype(jnp.int32), pl.ds(0, 8), :])))

            def keep_odd(j, g, job):
                h0, n = HEAD_GROUPS[g]
                for h in range(h0, h0 + 2 * n):
                    if buf:
                        carried[j, h] = both(p_acc[j], U, h)
                    else:
                        qkv_odd[j * H + h] = both(p_acc[j], U, h)
                job()

            order, ends = [], []
            for g in range(3):
                for j in range(3):
                    passes = proj_passes(ph, j, g)
                    order += product_jobs(passes, ph, (1 - ph,),
                                          (lambda l: ordered(mem_in(l))) if j or not last else None,
                                          tok_p, m_acc[j], p_acc[j]) or [None] * len(passes)
                    ends.append((len(order) + 8, j, g))
            passes = out_passes(ph)
            lag = [tile - 3 * NW >= NW - len(OUT[2]) for terms, _, _ in passes for _, tile in terms]
            delay, slope = LAST_HEADS_LAG[tune]
            jobs = product_jobs(passes, ph, o_halves, None if last else mem_o, tok_o, m_acc[3], o_acc)
            order += [jobs[i] for i in sorted(
                range(len(jobs)), key=lambda i: i + lag[i] * max(0, delay - i * slope / 100))]
            for at, j, g in ends if ph == T else ():
                order[at] = (order[at][0], functools.partial(keep_odd, j, g, order[at][1]))
            jobs = []
            for i, job in enumerate(order):
                for heads, s_at, v_at in zip(HEADS, SCORES_AT[tune], VALUES_AT[tune]):
                    jobs += [(True, functools.partial(scores, h)) for h in heads if i == s_at]
                    jobs += [(True, functools.partial(values, h)) for h in heads if i == v_at]
                jobs += [job] if job else []
            for job in [f for _, f in jobs] if last else _rounds(jobs):
                job()
                now[0] += 1
                if now[0] in fill:
                    due.append((0, fill.pop(now[0])()))
            assert not fill
            if not last:
                return real_tiles(lambda n: _take(m_acc[3], n))
            for _, job in product_jobs(out_passes(T), T, (), None, tok_o, None, o_acc):
                job()

        def add_attention(s, o_acc):
            total = _memo(lambda p: both(o_acc, p, NT))

            def job(p, k):
                x = x_tile(k, s + p) + (both(o_acc, p, k) + total(p))
                xs[k, s + p] = x.astype(BF16)
                return bits(x)

            return [functools.partial(job, p, k) for k in range(NT) for p in (T, U)]

        def first_step(li):
            def start_projection(j):
                prepare_proj(j)
                mem_in = memory_rows(mem0[...].astype(F32))
                for g in range(3):
                    acc = {}
                    for _, job in product_jobs(proj_passes(T, j, g), T, (), mem_in, None, acc, None):
                        job()
                    for h in sorted(acc):
                        qkv_even[j * H + h, pl.ds(0, M), :] = _take(acc, h)

            def project(j, tick=lambda: None):
                tok_p = token_rows(0)
                for g, (h0, n) in enumerate(HEAD_GROUPS):
                    acc = {}
                    for ph, halves in ((U, ()), (T, (0, 1))):
                        for _, job in product_jobs(proj_passes(ph, j, g), ph, halves, None, tok_p, None, acc):
                            job()
                            tick()
                    for h in range(h0, h0 + 2 * n):
                        qkv_even[j * H + h, pl.ds(M, SEG), :] = both(acc, T, h)
                        qkv_odd[j * H + h] = both(acc, U, h)

            def body(j, c):
                pl.when(li == 0)(lambda: start_projection(j))
                pl.when(li + j == 0)(lambda: wait_all(x_head))

                @pl.when(j == 0)
                def _():
                    for s in range(4):
                        attn_in(s & 2, s >> 1, s & 1)

                pl.when(j < 2)(lambda: project(j))
                return c

            lax.fori_loop(0, 3, body, 0)
            ps, now = {}, [0]

            def values(h, scale_first):
                p, inv = ps.pop(h)
                y = _dot(p * inv if scale_first else p, qkv_even[2 * H + h].astype(BF16))
                y = y if scale_first else y * inv
                o_mem[h], o_even0[h] = y[:M], y[M:]

            def tick():
                now[0] += 1
                for h in range(H):
                    if now[0] == 4 + 24 * (h // 4):
                        ps[h] = probs(qkv_even[h], qkv_even[H + h])
                    if now[0] == FIRST_VALUES_AT[h // 4]:
                        values(h, False)

            project(2, tick)
            for h in sorted(ps):
                values(h, True)
            pl.when(li == 0)(prepare_out)
            acc = {}
            for _, job in product_jobs(out_passes(T), T, (), lambda l: _combine(l, lambda h: o_mem[h]),
                                       None, acc, None):
                job()
            pl.when(li == 0)(lambda: wait_all(x_soon))
            return real_tiles(lambda n: _take(acc, n))

        def pair(t, buf, mem, carried, pending=(), rows_of=None, final=False):
            rows = [(p, r) for p in (T, U) for r in (0, HALF)]
            fill, p_acc, o_acc = {}, [{}, {}, {}], {}
            if not final:
                _spread(fill, [functools.partial(attn_in, 2 * t + 2, 1 - buf, p, r, HALF) for p, r in rows],
                        *SIDE_JOBS[buf][0])
            _spread(fill, [functools.partial(mixer_in, jnp.maximum(2 * t - 4 + p, p), r, HALF) for p, r in rows],
                    *SIDE_JOBS[buf][1])
            _spread(fill, prepare_mix(t - 3), *SIDE_JOBS[buf][2])
            _spread(fill, pending, 11, 100)
            zero = (t >> 16).astype(U32)
            tok_p = rows_of or token_rows(buf)
            mem = step(U, mem, buf, tok_p, p_acc, (0,), o_acc, {k: f for k, f in fill.items() if k < 700},
                       zero, carried)
            fill = {k - 699: f for k, f in fill.items() if k >= 700}
            tok_next = token_rows(1 - buf)
            if buf and not final:
                _spread(fill, [functools.partial(lambda l, hs: bits(jnp.concatenate([tok_next(l, h) for h in hs])),
                                                 terms[0][0], (0,) if shared else (0, 1))
                               for terms, _, shared in proj_passes(U, 0, 0)[:50]], 123, 400)
            mem = step(T, mem, buf, tok_p, p_acc, (1,), o_acc, fill, zero, carried)
            return mem, add_attention(2 * t - 2, o_acc), tok_next

        def two_pairs(li, i, mem):
            @pl.when((li == 0) & (2 * i + 1 == 3))
            def _():
                wait_all(x_rest + [w1_cp])
                w2_cp.start()

            pl.when((li == 0) & (2 * i + 1 == 3 + 2 * SLICES))(w2_cp.wait)
            carried = {}
            mem, pending, rows_of = pair(2 * i + 1, 1, mem, carried)
            mem, pending, _ = pair(2 * i + 2, 0, mem, carried, pending, rows_of)
            for job in pending:
                job()
            return mem

        def last_steps(li, mem):
            carried, fill, o_acc = {}, {}, {}
            zero = li >> 16
            mem, pending, _ = pair(NSEG // 2 - 1 + zero, 1, mem, carried, final=True)
            _spread(fill, pending, 11, 100)
            _spread(fill, [f for u in range(NSEG // 2 - 3, 4 * SLICES) for f in prepare_mix(u + zero)], 20, 328)
            _spread(fill, [functools.partial(mixer_in, NSEG - 4 + p, r, HALF) for p in (T, U) for r in (0, HALF)],
                    123, 340)
            tile = _memo(lambda g, k: h_tile(g, k, 0))
            _spread(fill, [functools.partial(fetch, *gk, tile) for gk in early], 60, 290)
            step(U, mem, 0, None, [{}, {}, {}], (0, 1), o_acc, fill, zero.astype(U32), carried, last=True)
            for job in add_attention(NSEG - 2, o_acc):
                job()
            mixer_in(NSEG - 2)
            mixer_in(NSEG - 1)

        def h_tile(g, k, i):
            return hb[i, pl.ds((8 * g + TOKEN_TILE[k]) * GB, GB)].reshape(128, 128).T

        def fetch(g, k, tile):
            h_next[g, 7 + k] = tile(g, k)
            h_next[g, k] = y = tile(g, k) + tile(g, 7)
            return bits(y[:32])

        def add_mixed(n, i, y):
            rows = pl.ds(n * GB, GB)
            x = pltpu.bitcast(xs.bitcast(U32)[i, rows].reshape(64, 128), BF16).astype(F32) + y.T
            xs[i, rows] = x.reshape(GB, SEG, 128).astype(BF16)
            return bits(x[-SEG:])

        def mix_weights(m, g, k):
            mirrored = (MIRROR[k[0]] if m else k[0], *k[1:])
            if mirrored in MIX_TILE:
                return pltpu.bitcast(wb.bitcast(U32)[(2 * m + g) * NB + MIX_TILE[mirrored]], BF16)
            (v, f), = MIX[mirrored][1]
            s, = _mix_block(v, f)
            return w12[m, pl.ds(f * 128, 128), pl.ds((8 * g + TOKEN_TILE[s]) * 128, 128)]

        def mixer(li, i, c):
            zero = (i >> 16).astype(U32)
            now, due, keys = [0], [], _mix_order()
            tile = _memo(lambda g, k: h_tile(g, k, i))
            next_tile = _memo(lambda g, k: h_tile(g, k, jnp.minimum(i + 1, NT - 1)))
            virtual = _memo(lambda g, v: h_next[g, v] if (g, v % 7) in early else
                            tile(g, v) + tile(g, 7) if v < 7 else tile(g, v - 7))

            def products(m, halves, get, done):
                left, acc = {n: 0 for n in range(NF)}, {}
                for k in keys:
                    for _, n in MIX[k][2]:
                        left[n] += 1
                for k in keys:
                    res = None
                    for g in halves:
                        a = _combine(MIX[k][0], lambda b: get(g, *b))
                        now[0] += 1
                        for at, f in due:
                            if at == now[0]:
                                a = jnp.concatenate([after(a[:8], f(), zero), a[8:]])
                        part = (_dot if m else _dot_nt)(a, mix_weights(m, g, k))
                        res = part if res is None else part + res
                    for key, sign in MIX[k][2].items():
                        _signed_add(acc, key, sign, res)
                        left[key[1]] -= 1
                        if not left[key[1]]:
                            done(key[1], jnp.concatenate([_take(acc, (p, key[1])) for p in (T, U)]))

            def activate(n, u):
                for r in range(0, 128, 32):
                    g_buf[n, pl.ds(r, 32), :] = _gelu(u[r:r + 32] + bias[0, :, pl.ds(n * 128, 128)])
                    y = bits(g_buf[n + zero.astype(jnp.int32), pl.ds(r, 8), :])
                    due.append((max([now[0] + 11] + [at + 8 for at, _ in due[required:]]), lambda y=y: y))

            def collect(g):
                left, acc = dict(enumerate([2] * 7 + [7])), {}

                def done(v, y):
                    for k in (v, 7) if v < 7 else (v - 7,):
                        _signed_add(acc, k, 1, y)
                        left[k] -= 1
                        if not left[k]:
                            n = 8 * g + TOKEN_TILE[k]
                            z = _take(acc, k) + bias[1, :, pl.ds(n * 128, 128)]
                            if n in late_y:
                                y_last[late_y.index(n)] = z
                            else:
                                add_mixed(n, i, z)

                return done

            def finish_previous(j):
                return add_mixed(late_y[j], jnp.maximum(i - 1, 0), jnp.where(i > 0, y_last[j], 0.0))

            due += [(20 + 9 * j, functools.partial(finish_previous, j)) for j in range(len(late_y))]
            due += [(208 + 34 * j, functools.partial(fetch, *gk, next_tile)) for j, gk in enumerate(early)]
            required = len(due)
            products(0, (0, 1), lambda g, p, v: virtual(g, v)[p * 64:(p + 1) * 64], activate)
            pl.when((li == 1) & (i > 0))(lambda: out_cp(i - 1, 1).start())
            for g in range(2):
                products(1, (g,), lambda _, p, f: g_buf[f, pl.ds(p * 64, 64), :], collect(g))
            assert all(at <= now[0] for at, _ in due[:required])
            pl.when(li == 1)(lambda: out_cp(i, 0).start())
            return c

        def layer(li, c):
            mem = lax.fori_loop(0, NSEG // 4 - 1, functools.partial(two_pairs, li), first_step(li))
            last_steps(li, mem)
            lax.fori_loop(0, NT, functools.partial(mixer, li), 0)
            for j, n in enumerate(late_y):
                add_mixed(n, NT - 1, y_last[j])
            return c

        start_all([w_cp(0, i) for i in range(COPIES_FIRST)] + small)
        w12[pl.ds(0, 2), pl.ds(F, NF * 128 - F), :] = jnp.zeros((2, NF * 128 - F, S), BF16)
        for f in range(NF):
            w12[2, pl.ds(f * 128, 16), pl.ds(0, S // 2)] = jnp.zeros((16, S // 2), BF16)
        y_last[...] = jnp.zeros(y_last.shape, F32)
        bias[0] = jnp.zeros((1, S), F32)
        wait_all(small)
        bias[0, :, pl.ds(0, F)] = b1[...].astype(F32).reshape(1, F)
        bias[1] = b2[...].astype(F32).reshape(1, S)
        lax.fori_loop(0, 2, layer, 0)
        out_cp(NT - 1, 1).start()
        wait_all([out_cp(i, part) for i in range(NT) for part in range(2)])

    hbm = pl.BlockSpec(memory_space=pltpu.MemorySpace.HBM)
    out = pl.pallas_call(
        kernel,
        out_shape=jax.ShapeDtypeStruct((NSEG, SEG, D), BF16),
        in_specs=[hbm] * 10,
        out_specs=hbm,
        scratch_shapes=[
            pltpu.VMEM((M, D), BF16),
            pltpu.VMEM((F,), BF16),
            pltpu.VMEM((S,), BF16),
            pltpu.VMEM((NT, NSEG, SEG, 128), BF16),
            pltpu.VMEM((3 * SLICES, NT, 18 * H, E), BF16),
            pltpu.VMEM((SLICES, H, 16, D), BF16),
            pltpu.VMEM((3, NF * 128, S), BF16),
            pltpu.VMEM((4 * NW, 128, 128), BF16),
            pltpu.VMEM((4 * NB, 128, 128), BF16),
            pltpu.VMEM((2, 1, S), F32),
            pltpu.VMEM((2, 2, NT + 1, SEG, 128), F32),
            pltpu.VMEM((3 * H, L, E), F32),
            pltpu.VMEM((3 * H, SEG, E), F32),
            pltpu.VMEM((H, M, E), F32),
            pltpu.VMEM((H, SEG, E), F32),
            pltpu.VMEM((H, SEG, E), F32),
            pltpu.VMEM((H, SEG, E), F32),
            pltpu.VMEM((NT, NSEG, SEG, 128), F32),
            pltpu.VMEM((2, 14, 128, 128), F32),
            pltpu.VMEM((NF, 128, 128), F32),
            pltpu.VMEM((len(late_y), 128, 128), F32),
            pltpu.SemaphoreType.DMA((3 * NT + 5,)),
            pltpu.SemaphoreType.DMA((4 * SLICES,)),
            pltpu.SemaphoreType.DMA((2 * NT,)),
        ],
        compiler_params=pltpu.CompilerParams(vmem_limit_bytes=112 * 1024 * 1024),
        name="rmt_mixer",
    )(
        A_x.reshape(NSEG, SEG, D), A_mem0.reshape(M, D),
        *[w.reshape(NT, SLICES, 16 * H, E) for w in (A_Wq, A_Wk, A_Wv)], A_Wo.reshape(H, SLICES, 16, D),
        B_w1.T, B_b1, B_w2, B_b2,
    )
    return out.reshape(A_x.shape)
```

```python
import functools
import math

import jax
import jax.numpy as jnp
from jax import lax
import jax.experimental.pallas as pl
import jax.experimental.pallas.tpu as pltpu

F32 = jnp.float32
BF16 = jnp.bfloat16
U32 = jnp.uint32
LOG2E = 1.4426950408889634
T, U = 0, 1
SLICES = 8


def _dot(a, b):
    return lax.dot_general(a, b, (((1,), (0,)), ((), ())), preferred_element_type=F32)


def _dot_nt(a, b):
    return lax.dot_general(a, b, (((1,), (1,)), ((), ())), preferred_element_type=F32)


def _layernorm(x):
    n = x.shape[-1]
    d = x - jnp.sum(x, axis=-1, keepdims=True) * (1.0 / n)
    v = jnp.sum(d * d, axis=-1, keepdims=True) * (1.0 / n)
    return d * lax.rsqrt(v + 1e-5)


def _gelu(x):
    c = math.sqrt(2.0 / math.pi)
    return 0.5 * x * (1.0 + jnp.tanh(c * (x + 0.044715 * (x * x * x))))


def _half_word(w, i):
    return lax.bitcast_convert_type(w & jnp.uint32(0xFFFF0000) if i else w << 16, F32)


def _memo(f):
    seen = {}

    def g(*k):
        if k not in seen:
            seen[k] = f(*k)
        return seen[k]

    return g


def _scheme(X, Y, pairs):
    P = {}
    for i, (a, d) in enumerate(X):
        ys = [Y[l] for k, l in pairs if k == i]
        P['m3', i] = ({(T, a): 1}, {(a, d): 1, **{(b, d): -1 for b, _ in ys}}, {(T, d): 1, (U, d): 1})
        P['m6', i] = ({(U, a): 1, (T, a): -1}, {(a, d): 1, **{(a, c): 1 for _, c in ys}}, {(U, d): 1})
    for l, (b, c) in enumerate(Y):
        xs = [X[i] for i, k in pairs if k == l]
        P['m4', l] = ({(U, b): 1}, {(b, c): 1, **{(a, c): -1 for a, _ in xs}}, {(T, c): 1, (U, c): 1})
        P['m7', l] = ({(T, b): 1, (U, b): -1}, {(b, c): 1, **{(b, d): 1 for _, d in xs}}, {(T, c): 1})
    for i, l in pairs:
        (a, d), (b, c) = X[i], Y[l]
        P['m1', i, l] = ({(T, a): 1, (U, b): 1}, {(a, c): 1, (b, d): 1}, {(T, c): 1, (U, d): 1})
        P['m2', i, l] = ({(U, a): 1, (U, b): 1}, {(a, c): 1}, {(U, c): 1, (U, d): -1})
        P['m5', i, l] = ({(T, a): 1, (T, b): 1}, {(b, d): 1}, {(T, c): -1, (T, d): 1})
    return P


HEAD_GROUPS = ((0, 6), (12, 5), (22, 5))
PAIRS = {6: [(i, l) for i in range(6) for l in range(6) if l not in (i, (i + 1) % 6)],
         5: [(i, l) for i in range(5) for l in range(5) if l != i]}
PROJ = [_scheme([(i, h + i) for i in range(n)], [(i, h + n + i) for i in range(n)], PAIRS[n])
        for h, n in HEAD_GROUPS]
OUT = [_scheme([(h + i, i) for i in range(n)], [(h + n + i, i) for i in range(n)], PAIRS[n])
       for h, n in HEAD_GROUPS]
ATTN_TILE = {k: i for i, k in enumerate((g, k) for g, s in enumerate(PROJ) for k in s)}


def _attn_block(v, h):
    r = 5 if h >= 12 else (h + 1) % 6 if h < 6 else (h - 1) % 6
    return {v: 1} if r == 5 else {r: 1} if v == 5 else {v: 1, r: -1}


_DIAG = [(i, i) for i in range(14)]
MIX = _scheme(_DIAG[:7], _DIAG[7:], [(i, l) for i in range(7) for l in range(7)])
MIX_TILE = {k: i for i, k in enumerate(k for k in MIX if k[0] not in ('m2', 'm5') or k[1] == k[2])}
TOKEN_TILE = (0, 1, 2, 3, 4, 5, 7, 6)
MIRROR = {'m1': 'm1', 'm2': 'm5', 'm5': 'm2', 'm3': 'm6', 'm6': 'm3', 'm4': 'm7', 'm7': 'm4'}


def _mix_block(v, f):
    if f < 7:
        return {7: 1} if v == f else {f: 1, 7: -1} if v == f + 7 else {v - 7: 1}
    rest = [k for k in range(7) if k != f - 7]
    if v == f - 7:
        return {7: 1, **{k: -1 for k in rest}}
    return {f - 7: 1, 7: -1, **{k: 1 for k in rest}} if v == f else {v: 1}


def _signed_add(acc, key, sign, val):
    if key not in acc:
        acc[key] = (sign, val)
        return
    s0, v0 = acc[key]
    acc[key] = (s0, v0 + val) if s0 == sign else (1, v0 - val if s0 > 0 else val - v0)


def _take(acc, key):
    s, v = acc[key]
    acc[key] = None
    assert s > 0
    return v


def _combine(terms, get):
    acc = {}
    for k, c in terms.items():
        _signed_add(acc, 0, c, get(k))
    return _take(acc, 0)


def _half_order(ph, n, mode):
    diag, single = (('m3', 'm7'), 'm5') if ph == T else (('m4', 'm6'), 'm2')
    pick = {'column': lambda p: p[ph], 'finish': min, 'open': max}[mode]
    left = [(d, s) for s in range(n) for d in diag]
    keys, done = [], 0
    for s in range(n):
        while mode == 'column' and left and left[0][1] <= s:
            keys.append(left.pop(0))
        for p in sorted((p for p in PAIRS[n] if pick(p) == s), key=lambda p: p[0] != s):
            keys += [(single, *p), ('m1', *p)]
            done += 1
            if mode != 'column' and done % 2 == 0 and left and (mode == 'finish' or left[0][1] <= s):
                keys.append(left.pop(0))
        while left and left[0][1] <= s:
            keys.append(left.pop(0))
    return keys


def _mix_order():
    keys = []
    for s in range(7):
        keys += [(m, s, l) for l in [*range(s + 1, 7), s] for m in ('m1', 'm2', 'm5')] + [('m3', s), ('m6', s)]
        keys += [(m, i, s) for i in range(s + 1, 7) for m in ('m1', 'm2', 'm5')] + [('m4', s), ('m7', s)]
    return keys


def _rounds(jobs):
    queues = [[(i, f) for i, (long, f) in enumerate(jobs) if long == k] for k in (False, True)]
    out = []
    while queues[0] or queues[1]:
        at = [q[min(3, len(q) - 1)][0] if q else math.inf for q in queues]
        q = queues[at[1] < at[0]]
        out += [f for _, f in q[:4]]
        del q[:4]
    return out


def _spread(fill, jobs, lo, hi):
    for i, f in enumerate(jobs):
        at = lo + i * (hi - lo) // len(jobs)
        while at in fill:
            at += 1
        fill[at] = f


HEADS = ((0, 1, 2, 3), (4, 5, 6, 7), (8, 9, 10, 11), (12, 13, 14, 15), (16, 17, 18, 19),
         (20, 21, 22, 27), (23, 28, 24, 29), (25, 30, 26, 31))
SCORES_AT = ((146, 152, 185, 290, 326, 446, 452, 462), (154, 152, 177, 303, 326, 462, 447, 459),
             (157, 152, 192, 305, 326, 444, 452, 462), (164, 152, 185, 305, 326, 446, 466, 460))
VALUES_AT = ((200, 225, 269, 395, 423, 496, 515, 509), (202, 225, 269, 395, 415, 496, 510, 520),
             (202, 225, 280, 395, 410, 487, 510, 520), (200, 225, 269, 385, 410, 496, 510, 517))
LAST_HEADS_LAG = ((65, 68), (72, 68), (65, 88), (65, 84))
SETTLE = ((31, 20), (30, 29), (30, 20), (30, 30))
SIDE_JOBS = (((230, 464), (800, 1135), (130, 542)), ((88, 470), (800, 1043), (22, 501)))
FIRST_VALUES_AT = (112, 136, 160, 208, 232, 0, 0, 0)
COPIES_FIRST, COPIES_AHEAD = 2, 6


@functools.partial(jax.jit, static_argnames=("A_seg_len",))
def pallas_interleave_layers__memory_aug_recurrent_mem_tr__mixer_token_mlp__prompt_kernel(
        A_x, A_mem0, A_Wq, A_Wk, A_Wv, A_Wo, A_seg_len, B_x, B_w1, B_b1, B_w2, B_b2):
    del B_x
    _, S, D = A_x.shape
    _, H, E = A_Wq.shape
    M = A_mem0.shape[1]
    SEG = int(A_seg_len)
    F = B_w1.shape[1]
    L, HALF, NSEG, GB = M + SEG, SEG // 2, S // SEG, 128 // SEG
    NT, NS, NF = D // 128, S // 128, -(-F // 128)
    NW, NB = len(ATTN_TILE), len(MIX_TILE)
    assert (D, H, E, M, SEG, S, NF) == (640, 32, 128, 8, 32, 2048, 14) and F % 16 == 0
    early = [(g, k) for k in range(6) for g in range(2)]
    late_y = (13, 14, 15)

    def proj_passes(ph, j, g):
        mode = 'column'
        if isinstance(j, int):
            mode = 'open' if (j, g) == (0, 0) else 'finish' if j and g == 2 else mode
        return [([(PROJ[g][k][0], NW * j + ATTN_TILE[g, k])], PROJ[g][k][2], k[0] == 'm1')
                for k in _half_order(ph, HEAD_GROUPS[g][1], mode)]

    def out_passes(ph):
        keys = [k for k in _half_order(ph, 6, 'finish') if 5 in k[1:]] + _half_order(ph, 5, 'finish')
        groups = {k: [g for g in range(3) if k in OUT[g]] for k in keys}
        return [([(OUT[g][k][0], 3 * NW + ATTN_TILE[g, k]) for g in gs], OUT[gs[0]][k][2], k[0] == 'm1')
                for k, gs in groups.items()]

    def kernel(x_hbm, mem0_hbm, wq_hbm, wk_hbm, wv_hbm, wo_hbm, w1_hbm, b1_hbm, w2_hbm, b2_hbm, out_hbm,
               mem0, b1, b2, xs, wqkv_in, wo_in, w12, wa, wb, bias, xn, qkv_even, qkv_odd, o_mem,
               o_even0, o_even1, o_odd, hb, h_next, g_buf, y_last, sems, wsems, osems):
        o_even = (o_even0, o_even1)

        def staged(n):
            return wqkv_in.at[n, :, pl.ds(0, 16 * H)]

        def w_cp(j, i):
            n = j * SLICES + i
            if j < 3:
                return pltpu.make_async_copy((wq_hbm, wk_hbm, wv_hbm)[j].at[:, i], staged(n), wsems.at[n])
            return pltpu.make_async_copy(wo_hbm.at[:, i], wo_in.at[i], wsems.at[n])

        def x_cps(i, lo, hi):
            return [pltpu.make_async_copy(x_hbm.at[pl.ds(lo, hi - lo), :, pl.ds(k * 128, 128)],
                                          xs.at[k, pl.ds(lo, hi - lo)], sems.at[i]) for k in range(NT)]

        def out_cp(i, part):
            cols = pl.ds(pl.multiple_of(i * 128, 128), 128)
            cut = late_y[0] * GB
            rows = (pl.ds(0, cut), pl.ds(cut, NSEG - cut))[part]
            return pltpu.make_async_copy(xs.at[i, rows], out_hbm.at[rows, :, cols], osems.at[2 * i + part])

        x_head, x_soon, x_rest = x_cps(0, 0, 4), x_cps(1, 4, 8), x_cps(2, 8, NSEG)
        w1_cp, w2_cp, *small = [
            pltpu.make_async_copy(src, dst, sems.at[3 + i]) for i, (src, dst) in enumerate((
                (w1_hbm, w12.at[0, pl.ds(0, F)]), (w2_hbm, w12.at[1, pl.ds(0, F)]),
                (mem0_hbm, mem0), (b1_hbm, b1), (b2_hbm, b2)))]

        def start_all(cps):
            for cp in cps:
                cp.start()

        def wait_all(cps):
            for cp in cps:
                cp.wait()

        def start_ahead(j, i):
            for k in range(4):
                @pl.when((j * SLICES + i + COPIES_AHEAD) // SLICES == k)
                def _():
                    w_cp(k, (i + COPIES_AHEAD) % SLICES).start()

        def weight_sums(m, i, schemes, block):
            def store(g, k, y):
                wa[NW * m + ATTN_TILE[g, k], pl.ds(pl.multiple_of(i * 16, 16), 16), :] = y.astype(BF16)

            for g, (scheme, (_, n)) in enumerate(zip(schemes, HEAD_GROUPS)):
                acc = {}
                for a, b in PAIRS[n]:
                    for name in ('m2', 'm5', 'm1'):
                        store(g, (name, a, b), _combine(scheme[name, a, b][1], lambda k: block(*k)))
                    for k in (('m3', a), ('m6', a), ('m4', b), ('m7', b)):
                        w = scheme[k][1]
                        new = [x for x in w if x in scheme['m1', a, b][1]]
                        for x in new if k in acc else [next(iter(w))] + new:
                            _signed_add(acc, k, w[x], block(*x))
                        if (a, b) == [p for p in PAIRS[n] if p[k[0] in ('m4', 'm7')] == k[1]][-1]:
                            store(g, k, _take(acc, k))

        def prepare_proj(j):
            words = wqkv_in.bitcast(U32)

            def body(i, c):
                n = j * SLICES + i
                pltpu.make_async_copy(staged(n), staged(n), wsems.at[n]).wait()
                pl.when(n == 0)(lambda: start_all(
                    [w_cp(0, k) for k in range(COPIES_FIRST, COPIES_AHEAD)] + x_head))
                start_ahead(j, i)
                word = _memo(lambda k, hp: jnp.concatenate(
                    [words[n, k, pl.ds(r * 4 * H + hp, 8, stride=H // 2), :] for r in range(2)]))
                real = _memo(lambda k, h: _half_word(word(k, h // 2), h % 2))
                weight_sums(j, i, PROJ, _memo(lambda v, h: _combine(_attn_block(v, h), lambda k: real(k, h))))
                return c

            lax.fori_loop(0, SLICES, body, 0)

        def prepare_out():
            def body(i, c):
                w_cp(3, i).wait()
                start_ahead(3, i)
                pl.when(i == 2)(lambda: start_all(x_soon))
                real = _memo(lambda h, n: wo_in[i, h, :, pl.ds(n * 128, 128)].astype(F32))
                weight_sums(3, i, OUT, _memo(lambda h, v: _combine(_attn_block(v, h), lambda n: real(h, n))))
                return c

            lax.fori_loop(0, SLICES, body, 0)
            start_all(x_rest + [w1_cp])

        def prepare_mix(u):
            half, i = jnp.maximum(u, 0) >> 3, jnp.maximum(u, 0) & 7
            sign = lax.convert_element_type((half & 2) - 1, F32)
            src = w12.at[jnp.where(u < 0, 2, half >> 1), pl.ds(pl.multiple_of(i * 16, 16), (NF - 1) * 128 + 16),
                         pl.ds(pl.multiple_of((half & 1) * (S // 2), S // 2), S // 2)]
            dst = wb.at[pl.ds(half * NB, NB), pl.ds(pl.multiple_of(i * 16, 16), 16)]
            word = _memo(lambda k, f: src[pl.ds(f * 128, 16), pl.ds(TOKEN_TILE[k] * 128, 128)])
            real = lambda k, f: word(k, f).astype(F32)
            total = _memo(lambda f: _combine({k: 1 for k in range(7)}, lambda k: real(k, f)))

            @_memo
            def block(v, f):
                if f >= 7 and v == f:
                    return total(f) - real(7, f)
                if v == f - 7:
                    return real(v, f) - block(f, f)
                return _combine(_mix_block(v, f), lambda k: real(k, f))

            def job(keys):
                done = []
                for k in keys:
                    (head, _), *tail = MIX[k][1].items()
                    y = block(*head)
                    if tail:
                        z = real(7, head[1]) if k[0] == 'm4' else _combine(
                            {b: 1 for b, _ in tail}, lambda b: block(*b))
                        y = y + z if k[0] == 'm1' else y + sign * z if tail[0][1] < 0 else y - sign * z
                    dst[MIX_TILE[k]] = y.astype(BF16)
                    done.append(bits(y[8:]))
                return functools.reduce(jnp.bitwise_or, done)

            off = [k for k in MIX_TILE if len(k) == 3 and k[1] != k[2]]
            parts = [p for d in range(7) for p in (
                [(x, d, d) for x in ('m2', 'm5', 'm1')], *[[(x, d)] for x in ('m3', 'm6', 'm4', 'm7')])]
            return [functools.partial(job, p) for p in parts + [off[c:c + 3] for c in range(0, len(off), 3)]]

        def bits(y):
            parts = [y[r:r + 8, c:c + 128] for r in range(0, y.shape[0], 8) for c in sorted({0, y.shape[1] - 128})]
            return functools.reduce(jnp.bitwise_or, [lax.bitcast_convert_type(p, U32) for p in parts])

        def after(y, done, zero):
            return lax.bitcast_convert_type(lax.bitcast_convert_type(y, U32) | (done & zero), F32)

        def tiles_and_sum(y):
            tiles = [y[:, k * 128:(k + 1) * 128] for k in range(NT)]
            return tiles + [functools.reduce(jnp.add, tiles)]

        def real_tiles(get):
            total = get(NT)
            return jnp.concatenate([get(n) + total for n in range(NT)], axis=1)

        def x_tile(k, s, r=0, n=SEG):
            return pltpu.bitcast(xs.bitcast(U32)[k, s, pl.ds(r // 2, n // 2), :], BF16).astype(F32)

        def load_x(s, r, n):
            return jnp.concatenate([x_tile(k, s, r, n) for k in range(NT)], axis=1)

        def attn_in(s, buf, p, r=0, n=SEG):
            y = tiles_and_sum(_layernorm(load_x(s + p, r, n)))
            for k, tile in enumerate(y):
                xn[buf, p, k, pl.ds(r, n), :] = tile
            return bits(y[-1])

        def mixer_in(s, r=0, n=SEG):
            y = _layernorm(_layernorm(load_x(s, r, n)))
            for k in range(NT):
                hb[k, s, pl.ds(r, n), :] = y[:, k * 128:(k + 1) * 128]
            return bits(y)

        def product_jobs(passes, ph, halves, mem_in, tok_in, mem_acc, tok_acc):
            jobs = []
            for terms, out, shared in passes:
                hs = () if tok_in is None else halves if shared else (0, 1)
                if mem_in is None and not hs:
                    continue

                def job(rows_of, tile, count, out, hs, parts):
                    rows = [mem_in({k: c for (p, k), c in rows_of.items() if p == ph})] if mem_in else []
                    rows += [tok_in(rows_of, h) for h in hs]
                    res = _dot(jnp.concatenate(rows), pltpu.bitcast(wa.bitcast(U32)[tile], BF16))
                    parts.append(res + parts[-1] if parts else res)
                    if len(parts) < count:
                        return
                    r0 = M if mem_in else 0
                    for (p, n), c in out.items():
                        if mem_in and p == ph:
                            _signed_add(mem_acc, n, c, parts[-1][:M])
                    for i, h in enumerate(hs):
                        for (p, n), c in out.items():
                            _signed_add(tok_acc, (p, n, h), c, parts[-1][r0 + i * HALF:r0 + (i + 1) * HALF])

                parts = []
                jobs += [(len(hs) > 1, functools.partial(job, *t, len(terms), out, hs, parts)) for t in terms]
            return jobs

        def memory_rows(mem):
            tiles = tiles_and_sum(mem)
            rows = _memo(lambda *l: _combine(dict(l), tiles.__getitem__))
            return lambda l: rows(*sorted(l.items()))

        def token_rows(buf):
            rows = _memo(lambda h, *l: _combine(dict(l), lambda k: xn[buf, k[0], k[1], pl.ds(h * HALF, HALF), :]))
            return lambda l, h: rows(h, *sorted(l.items()))

        def both(acc, p, n):
            return jnp.concatenate([_take(acc, (p, n, i)) for i in range(2)])

        def probs(q, k):
            sc = _dot_nt(q, k.astype(BF16)) * (E ** -0.5 * LOG2E)
            r = lax.broadcasted_iota(jnp.int32, (L, L), 0)
            c = lax.broadcasted_iota(jnp.int32, (L, L), 1)
            sc = jnp.where(((r < M) | (r >= c))[L - q.shape[0]:], sc, -1e9 * LOG2E)
            p = jnp.exp2(sc - jnp.max(sc, axis=-1, keepdims=True))
            total = jnp.sum(p, axis=-1, keepdims=True)
            inv = pltpu.reciprocal(total, approx=True)
            return p, inv * (2.0 - total * inv)

        def step(ph, mem, buf, tok_p, p_acc, o_halves, o_acc, fill, zero, carried, last=False):
            tune = 2 * buf + ph
            o_tok, o_dst = (o_even[1 - buf], o_odd), (o_even[buf], o_odd)[ph]
            m_acc, ps, seen, due = [{}, {}, {}, {}], {}, set(), []
            now = [0]
            mem_in = memory_rows(mem)

            def ordered(y):
                for e in [e for e in due if e[0] <= now[0]]:
                    y = after(y, e[1], zero)
                due[:] = [e for e in due if e[0] > now[0]]
                return y

            def mem_o(l):
                assert seen.issuperset(l)
                return ordered(_combine(l, lambda h: o_mem[h]))

            def tok_o(l, i):
                assert seen.issuperset(h for p, h in l if p == U == ph)
                return _combine(l, lambda k: o_tok[k[0]][k[1], pl.ds(i * HALF, HALF), :])

            def qkv(j, h):
                rows = [_take(m_acc[j], h)] if j or not last else []
                if ph == T:
                    return jnp.concatenate(rows + [both(p_acc[j], T, h)])
                return jnp.concatenate(rows + [carried.pop((j, h)) if carried else qkv_odd[j * H + h]])

            def scores(h):
                ps[h] = probs(qkv(0, h), qkv(1, h))

            def values(h):
                p, inv = ps.pop(h)
                y = _dot(p, qkv(2, h).astype(BF16)) * inv
                o_dst[h] = y[-SEG:]
                seen.add(h)
                if last:
                    return
                o_mem[h] = y[:M]
                if len(seen) % 4 == 0 and len(seen) <= SETTLE[tune][1]:
                    for ref in (o_dst, o_mem):
                        due.append((now[0] + SETTLE[tune][0], bits(ref[h + zero.astype(jnp.int32), pl.ds(0, 8), :])))

            def keep_odd(j, g, job):
                h0, n = HEAD_GROUPS[g]
                for h in range(h0, h0 + 2 * n):
                    if buf:
                        carried[j, h] = both(p_acc[j], U, h)
                    else:
                        qkv_odd[j * H + h] = both(p_acc[j], U, h)
                job()

            order, ends = [], []
            for g in range(3):
                for j in range(3):
                    passes = proj_passes(ph, j, g)
                    order += product_jobs(passes, ph, (1 - ph,),
                                          (lambda l: ordered(mem_in(l))) if j or not last else None,
                                          tok_p, m_acc[j], p_acc[j]) or [None] * len(passes)
                    ends.append((len(order) + 8, j, g))
            passes = out_passes(ph)
            lag = [tile - 3 * NW >= NW - len(OUT[2]) for terms, _, _ in passes for _, tile in terms]
            delay, slope = LAST_HEADS_LAG[tune]
            jobs = product_jobs(passes, ph, o_halves, None if last else mem_o, tok_o, m_acc[3], o_acc)
            order += [jobs[i] for i in sorted(
                range(len(jobs)), key=lambda i: i + lag[i] * max(0, delay - i * slope / 100))]
            for at, j, g in ends if ph == T else ():
                order[at] = (order[at][0], functools.partial(keep_odd, j, g, order[at][1]))
            jobs = []
            for i, job in enumerate(order):
                for heads, s_at, v_at in zip(HEADS, SCORES_AT[tune], VALUES_AT[tune]):
                    jobs += [(True, functools.partial(scores, h)) for h in heads if i == s_at]
                    jobs += [(True, functools.partial(values, h)) for h in heads if i == v_at]
                jobs += [job] if job else []
            for job in [f for _, f in jobs] if last else _rounds(jobs):
                job()
                now[0] += 1
                if now[0] in fill:
                    due.append((0, fill.pop(now[0])()))
            assert not fill
            if not last:
                return real_tiles(lambda n: _take(m_acc[3], n))
            for _, job in product_jobs(out_passes(T), T, (), None, tok_o, None, o_acc):
                job()

        def add_attention(s, o_acc):
            total = _memo(lambda p: both(o_acc, p, NT))

            def job(p, k):
                x = x_tile(k, s + p) + (both(o_acc, p, k) + total(p))
                xs[k, s + p] = x.astype(BF16)
                return bits(x)

            return [functools.partial(job, p, k) for k in range(NT) for p in (T, U)]

        def first_step(li):
            def start_projection(j):
                prepare_proj(j)
                mem_in = memory_rows(mem0[...].astype(F32))
                for g in range(3):
                    acc = {}
                    for _, job in product_jobs(proj_passes(T, j, g), T, (), mem_in, None, acc, None):
                        job()
                    for h in sorted(acc):
                        qkv_even[j * H + h, pl.ds(0, M), :] = _take(acc, h)

            def project(j, tick=lambda: None):
                tok_p = token_rows(0)
                for g, (h0, n) in enumerate(HEAD_GROUPS):
                    acc = {}
                    for ph, halves in ((U, ()), (T, (0, 1))):
                        for _, job in product_jobs(proj_passes(ph, j, g), ph, halves, None, tok_p, None, acc):
                            job()
                            tick()
                    for h in range(h0, h0 + 2 * n):
                        qkv_even[j * H + h, pl.ds(M, SEG), :] = both(acc, T, h)
                        qkv_odd[j * H + h] = both(acc, U, h)

            def body(j, c):
                pl.when(li == 0)(lambda: start_projection(j))
                pl.when(li + j == 0)(lambda: wait_all(x_head))

                @pl.when(j == 0)
                def _():
                    for s in range(4):
                        attn_in(s & 2, s >> 1, s & 1)

                pl.when(j < 2)(lambda: project(j))
                return c

            lax.fori_loop(0, 3, body, 0)
            ps, now = {}, [0]

            def values(h, scale_first):
                p, inv = ps.pop(h)
                y = _dot(p * inv if scale_first else p, qkv_even[2 * H + h].astype(BF16))
                y = y if scale_first else y * inv
                o_mem[h], o_even0[h] = y[:M], y[M:]

            def tick():
                now[0] += 1
                for h in range(H):
                    if now[0] == 4 + 24 * (h // 4):
                        ps[h] = probs(qkv_even[h], qkv_even[H + h])
                    if now[0] == FIRST_VALUES_AT[h // 4]:
                        values(h, False)

            project(2, tick)
            for h in sorted(ps):
                values(h, True)
            pl.when(li == 0)(prepare_out)
            acc = {}
            for _, job in product_jobs(out_passes(T), T, (), lambda l: _combine(l, lambda h: o_mem[h]),
                                       None, acc, None):
                job()
            pl.when(li == 0)(lambda: wait_all(x_soon))
            return real_tiles(lambda n: _take(acc, n))

        def pair(t, buf, mem, carried, pending=(), rows_of=None, final=False):
            rows = [(p, r) for p in (T, U) for r in (0, HALF)]
            fill, p_acc, o_acc = {}, [{}, {}, {}], {}
            if not final:
                _spread(fill, [functools.partial(attn_in, 2 * t + 2, 1 - buf, p, r, HALF) for p, r in rows],
                        *SIDE_JOBS[buf][0])
            _spread(fill, [functools.partial(mixer_in, jnp.maximum(2 * t - 4 + p, p), r, HALF) for p, r in rows],
                    *SIDE_JOBS[buf][1])
            _spread(fill, prepare_mix(t - 3), *SIDE_JOBS[buf][2])
            _spread(fill, pending, 11, 120)
            zero = (t >> 16).astype(U32)
            tok_p = rows_of or token_rows(buf)
            mem = step(U, mem, buf, tok_p, p_acc, (0,), o_acc, {k: f for k, f in fill.items() if k < 700},
                       zero, carried)
            fill = {k - 699: f for k, f in fill.items() if k >= 700}
            tok_next = token_rows(1 - buf)
            if buf and not final:
                def sum_rows(l, hs):
                    return bits(jnp.concatenate([tok_next(l, h)[8:] for h in hs]))

                _spread(fill, [functools.partial(sum_rows, terms[0][0], (0,) if shared else (0, 1))
                               for terms, _, shared in proj_passes(U, 0, 0)[:50]], 102, 400)
            mem = step(T, mem, buf, tok_p, p_acc, (1,), o_acc, fill, zero, carried)
            return mem, add_attention(2 * t - 2, o_acc), tok_next

        def two_pairs(li, i, mem):
            @pl.when((li == 0) & (2 * i + 1 == 3))
            def _():
                rest = xs.at[:, pl.ds(8, NSEG - 8)]
                wait_all([pltpu.make_async_copy(rest, rest, sems.at[2]), w1_cp])
                w2_cp.start()

            pl.when((li == 0) & (2 * i + 1 == 3 + 2 * SLICES))(w2_cp.wait)
            carried = {}
            mem, pending, rows_of = pair(2 * i + 1, 1, mem, carried)
            mem, pending, _ = pair(2 * i + 2, 0, mem, carried, pending, rows_of)
            for job in pending:
                job()
            return mem

        def last_steps(li, mem):
            carried, fill, o_acc = {}, {}, {}
            zero = li >> 16
            mem, pending, _ = pair(NSEG // 2 - 1 + zero, 1, mem, carried, final=True)
            _spread(fill, pending, 11, 100)
            _spread(fill, [f for u in range(NSEG // 2 - 3, 4 * SLICES) for f in prepare_mix(u + zero)], 20, 328)
            _spread(fill, [functools.partial(mixer_in, NSEG - 4 + p, r, HALF) for p in (T, U) for r in (0, HALF)],
                    123, 344)
            tile = _memo(lambda g, k: h_tile(g, k, 0))
            _spread(fill, [functools.partial(fetch, *gk, tile) for gk in early], 60, 255)
            step(U, mem, 0, None, [{}, {}, {}], (0, 1), o_acc, fill, zero.astype(U32), carried, last=True)
            for job in add_attention(NSEG - 2, o_acc):
                job()
            mixer_in(NSEG - 2)
            mixer_in(NSEG - 1)

        def h_tile(g, k, i):
            return hb[i, pl.ds((8 * g + TOKEN_TILE[k]) * GB, GB)].reshape(128, 128).T

        def fetch(g, k, tile):
            h_next[g, 7 + k] = tile(g, k)
            h_next[g, k] = y = tile(g, k) + tile(g, 7)
            return bits(y[:32])

        def add_mixed(n, i, y):
            rows = pl.ds(n * GB, GB)
            x = pltpu.bitcast(xs.bitcast(U32)[i, rows].reshape(64, 128), BF16).astype(F32) + y.T
            xs[i, rows] = x.reshape(GB, SEG, 128).astype(BF16)
            return bits(x[-SEG:])

        def mix_weights(m, g, k):
            mirrored = (MIRROR[k[0]] if m else k[0], *k[1:])
            if mirrored in MIX_TILE:
                return pltpu.bitcast(wb.bitcast(U32)[(2 * m + g) * NB + MIX_TILE[mirrored]], BF16)
            (v, f), = MIX[mirrored][1]
            s, = _mix_block(v, f)
            return w12[m, pl.ds(f * 128, 128), pl.ds((8 * g + TOKEN_TILE[s]) * 128, 128)]

        def mixer(li, i, c):
            zero = (i >> 16).astype(U32)
            now, due, keys = [0], [], _mix_order()
            tile = _memo(lambda g, k: h_tile(g, k, i))
            next_tile = _memo(lambda g, k: h_tile(g, k, jnp.minimum(i + 1, NT - 1)))
            virtual = _memo(lambda g, v: h_next[g, v] if (g, v % 7) in early else
                            tile(g, v) + tile(g, 7) if v < 7 else tile(g, v - 7))

            def products(m, halves, get, done):
                left, acc = {n: 0 for n in range(NF)}, {}
                for k in keys:
                    for _, n in MIX[k][2]:
                        left[n] += 1
                for k in keys:
                    res = None
                    for g in halves:
                        a = _combine(MIX[k][0], lambda b: get(g, *b))
                        now[0] += 1
                        for at, f in due:
                            if at == now[0]:
                                a = jnp.concatenate([after(a[:8], f(), zero), a[8:]])
                        part = (_dot if m else _dot_nt)(a, mix_weights(m, g, k))
                        res = part if res is None else part + res
                    for key, sign in MIX[k][2].items():
                        _signed_add(acc, key, sign, res)
                        left[key[1]] -= 1
                        if not left[key[1]]:
                            done(key[1], jnp.concatenate([_take(acc, (p, key[1])) for p in (T, U)]))

            def activate(n, u):
                for r in range(0, 128, 32):
                    g_buf[n, pl.ds(r, 32), :] = _gelu(u[r:r + 32] + bias[0, :, pl.ds(n * 128, 128)])
                    y = bits(g_buf[n + zero.astype(jnp.int32), pl.ds(r, 8), :])
                    due.append((max([now[0] + 11] + [at + 8 for at, _ in due[required:]]), lambda y=y: y))

            def collect(g):
                left, acc = dict(enumerate([2] * 7 + [7])), {}

                def done(v, y):
                    for k in (v, 7) if v < 7 else (v - 7,):
                        _signed_add(acc, k, 1, y)
                        left[k] -= 1
                        if not left[k]:
                            n = 8 * g + TOKEN_TILE[k]
                            z = _take(acc, k) + bias[1, :, pl.ds(n * 128, 128)]
                            if n in late_y:
                                y_last[late_y.index(n)] = z
                            else:
                                add_mixed(n, i, z)

                return done

            def finish_previous(j):
                return add_mixed(late_y[j], jnp.maximum(i - 1, 0), jnp.where(i > 0, y_last[j], 0.0))

            due += [(20 + 9 * j, functools.partial(finish_previous, j)) for j in range(len(late_y))]
            due += [(208 + 34 * j, functools.partial(fetch, *gk, next_tile)) for j, gk in enumerate(early)]
            required = len(due)
            products(0, (0, 1), lambda g, p, v: virtual(g, v)[p * 64:(p + 1) * 64], activate)
            pl.when((li == 1) & (i > 0))(lambda: out_cp(i - 1, 1).start())
            for g in range(2):
                products(1, (g,), lambda _, p, f: g_buf[f, pl.ds(p * 64, 64), :], collect(g))
            assert all(at <= now[0] for at, _ in due[:required])
            pl.when(li == 1)(lambda: out_cp(i, 0).start())
            return c

        def layer(li, c):
            mem = lax.fori_loop(0, NSEG // 4 - 1, functools.partial(two_pairs, li), first_step(li))
            last_steps(li, mem)
            lax.fori_loop(0, NT, functools.partial(mixer, li), 0)
            for j, n in enumerate(late_y):
                add_mixed(n, NT - 1, y_last[j])
            return c

        start_all([w_cp(0, i) for i in range(COPIES_FIRST)] + small)
        w12[pl.ds(0, 2), pl.ds(F, NF * 128 - F), :] = jnp.zeros((2, NF * 128 - F, S), BF16)
        for f in range(NF):
            w12[2, pl.ds(f * 128, 16), pl.ds(0, S // 2)] = jnp.zeros((16, S // 2), BF16)
        y_last[...] = jnp.zeros(y_last.shape, F32)
        bias[0] = jnp.zeros((1, S), F32)
        wait_all(small)
        bias[0, :, pl.ds(0, F)] = b1[...].astype(F32).reshape(1, F)
        bias[1] = b2[...].astype(F32).reshape(1, S)
        lax.fori_loop(0, 2, layer, 0)
        out_cp(NT - 1, 1).start()
        wait_all([out_cp(i, part) for i in range(NT) for part in range(2)])

    hbm = pl.BlockSpec(memory_space=pltpu.MemorySpace.HBM)
    out = pl.pallas_call(
        kernel,
        out_shape=jax.ShapeDtypeStruct((NSEG, SEG, D), BF16),
        in_specs=[hbm] * 10,
        out_specs=hbm,
        scratch_shapes=[
            pltpu.VMEM((M, D), BF16),
            pltpu.VMEM((F,), BF16),
            pltpu.VMEM((S,), BF16),
            pltpu.VMEM((NT, NSEG, SEG, 128), BF16),
            pltpu.VMEM((3 * SLICES, NT, 18 * H, E), BF16),
            pltpu.VMEM((SLICES, H, 16, D), BF16),
            pltpu.VMEM((3, NF * 128, S), BF16),
            pltpu.VMEM((4 * NW, 128, 128), BF16),
            pltpu.VMEM((4 * NB, 128, 128), BF16),
            pltpu.VMEM((2, 1, S), F32),
            pltpu.VMEM((2, 2, NT + 1, SEG, 128), F32),
            pltpu.VMEM((3 * H, L, E), F32),
            pltpu.VMEM((3 * H, SEG, E), F32),
            pltpu.VMEM((H, M, E), F32),
            pltpu.VMEM((H, SEG, E), F32),
            pltpu.VMEM((H, SEG, E), F32),
            pltpu.VMEM((H, SEG, E), F32),
            pltpu.VMEM((NT, NSEG, SEG, 128), F32),
            pltpu.VMEM((2, 14, 128, 128), F32),
            pltpu.VMEM((NF, 128, 128), F32),
            pltpu.VMEM((len(late_y), 128, 128), F32),
            pltpu.SemaphoreType.DMA((8,)),
            pltpu.SemaphoreType.DMA((4 * SLICES,)),
            pltpu.SemaphoreType.DMA((2 * NT,)),
        ],
        compiler_params=pltpu.CompilerParams(vmem_limit_bytes=112 * 1024 * 1024),
        name="rmt_mixer",
    )(
        A_x.reshape(NSEG, SEG, D), A_mem0.reshape(M, D),
        *[w.reshape(NT, SLICES, 16 * H, E) for w in (A_Wq, A_Wk, A_Wv)], A_Wo.reshape(H, SLICES, 16, D),
        B_w1.T, B_b1, B_w2, B_b2,
    )
    return out.reshape(A_x.shape)
```
